```python
import jax
import jax.numpy as jnp

def _softmax(x, axis=-1):
    return jax.nn.softmax(x, axis=axis)

def _gelu(x):
    return jax.nn.gelu(x, approximate=True)

def _silu(x):
    return jax.nn.silu(x)

def _sigmoid(x):
    return jax.nn.sigmoid(x)

def _layernorm(x, axis=-1, eps=1e-05):
    m = jnp.mean(x, axis=axis, keepdims=True)
    v = jnp.var(x, axis=axis, keepdims=True)
    return (x - m) / jnp.sqrt(v + eps)

def _scatter_add(tgt, idx, src, axis=0):
    return tgt.at[idx].add(src)

def _segment_sum(src, seg, n):
    return jax.ops.segment_sum(src, seg, n)

class _Rng:

    def __init__(self, key):
        self._k = key

    def _next(self):
        self._k, sub = jax.random.split(self._k)
        return sub

    def normal(self, shape):
        return jax.random.normal(self._next(), shape, dtype=jnp.bfloat16)

    def randint(self, lo, hi, shape):
        return jax.random.randint(self._next(), shape, lo, hi, dtype=jnp.int32)

    def uniform(self, shape, lo=0.0, hi=1.0):
        return jax.random.uniform(self._next(), shape, jnp.bfloat16, lo, hi)

    def permutation(self, n):
        return jax.random.permutation(self._next(), n)
kernel_name = 'adaLN_cond__ssm_conv_h3__mixer_s_mlp__prompt'

def setup_inputs():
    _rng = _Rng(jax.random.key(int.from_bytes(__import__("os").urandom(4), "little")))
    _w = lambda a: (lambda t: t.astype(jnp.bfloat16) if jnp.issubdtype(t.dtype, jnp.floating) else t)(jnp.asarray(a))

    def _A_setup():
        B, S, D = (1, 2048, 640)
        ks = 4
        return {'q': _w((lambda *s: _rng.normal(s) * 0.05)(B, S, D)), 'k': _w((lambda *s: _rng.normal(s) * 0.05)(B, S, D)), 'v': _w((lambda *s: _rng.normal(s) * 0.05)(B, S, D)), 'shift_k': _w((lambda *s: _rng.normal(s) * 0.05)(D, ks) * 0.5), 'ssm_k': _w((lambda *s: _rng.normal(s) * 0.05)(D, S) * (1.0 / S ** 0.5)), 'ssm_D': _w((lambda *s: _rng.normal(s) * 0.05)(D))}
    _A_in = _A_setup()

    def _B_setup():
        B, S, D, F = (1, 2048, 640, 1728)
        return {'x': _w((lambda *s: _rng.normal(s) * 0.05)(B, S, D)), 'w1': _w((lambda *s: _rng.normal(s) * 0.05)(D, D) * D ** (-0.5)), 'w2': _w((lambda *s: _rng.normal(s) * 0.05)(D, D) * D ** (-0.5)), 'w3': _w((lambda *s: _rng.normal(s) * 0.05)(D, F) * D ** (-0.5)), 'w4': _w((lambda *s: _rng.normal(s) * 0.05)(F, D) * F ** (-0.5))}
    _B_in = _B_setup()
    return {'A_q': _A_in['q'], 'A_k': _A_in['k'], 'A_v': _A_in['v'], 'A_shift_k': _A_in['shift_k'], 'A_ssm_k': _A_in['ssm_k'], 'A_ssm_D': _A_in['ssm_D'], 'B_x': _B_in['x'], 'B_w1': _B_in['w1'], 'B_w2': _B_in['w2'], 'B_w3': _B_in['w3'], 'B_w4': _B_in['w4'], 'c': _w((lambda *s: _rng.normal(s) * 0.05)(1, 640)), 'w_mod': _w((lambda *s: _rng.normal(s) * 0.05)(640, 6 * 640) * 640 ** (-0.5))}

def reference(A_q, A_k, A_v, A_shift_k, A_ssm_k, A_ssm_D, B_x, B_w1, B_w2, B_w3, B_w4, c, w_mod):

    def _A_ref(q, k, v, shift_k, ssm_k, ssm_D):
        B, S, D = q.shape
        ks = shift_k.shape[-1]
        k_pad = jnp.pad(k, ((0, 0), (ks - 1, 0), (0, 0)))
        k_shift = jnp.zeros_like(k)
        for t in range(ks):
            k_shift = k_shift + k_pad[:, t:t + S, :] * shift_k[:, ks - 1 - t][None, None, :]
        kv = k_shift * v
        L = 2 * S
        kv_pad = jnp.pad(kv, ((0, 0), (0, S), (0, 0)))
        kf_pad = jnp.pad(ssm_k, ((0, 0), (0, S)))
        kv_f = (lambda x, axes=(-2, -1): jnp.fft.rfft2(x.astype(jnp.float32), axes=axes))(kv_pad[:, None, :, :], axes=(1, 2))
        kf_f = (lambda x, axes=(-2, -1): jnp.fft.rfft2(x.astype(jnp.float32), axes=axes))(kf_pad[:, None, :], axes=(1, 2))
        kf_f = (lambda x, *d: x.transpose(*d))(kf_f, 1, 2, 0)
        y_f = kv_f * kf_f[None, :, :, :]
        y = (lambda x, s, axes=(-2, -1): jnp.fft.irfft2(x, s=s, axes=axes).astype(jnp.bfloat16))(y_f, (1, L), axes=(1, 2))[:, 0, :S, :]
        y = y + kv * ssm_D[None, None, :]
        return q * y

    def _B_ref(x, w1, w2, w3, w4):
        B, S, D = x.shape
        h = _gelu(_layernorm(x, axis=-1) @ w1)
        c = D // 4
        g0 = jnp.pad(h[:, :, 0 * c:1 * c], ((0, 0), (1, 0), (0, 0)))[:, :S, :]
        g1 = jnp.pad(h[:, :, 1 * c:2 * c], ((0, 0), (0, 1), (0, 0)))[:, 1:, :]
        g2 = jnp.pad(h[:, :, 2 * c:3 * c], ((0, 0), (2, 0), (0, 0)))[:, :S, :]
        g3 = jnp.pad(h[:, :, 3 * c:], ((0, 0), (0, 2), (0, 0)))[:, 2:, :]
        hs = jnp.concatenate([g0, g1, g2, g3], axis=-1) @ w2
        x1 = x + hs
        h2 = _gelu(_layernorm(x1, axis=-1) @ w3) @ w4
        return x1 + h2
    x = A_q
    mod = (_silu(c) @ w_mod).reshape(c.shape[0], 6, 1, -1)
    sa, ca, ga, sb, cb, gb = (mod[:, 0].copy(), mod[:, 1].copy(), mod[:, 2].copy(), mod[:, 3].copy(), mod[:, 4].copy(), mod[:, 5].copy())
    h = _layernorm(x, axis=-1) * (1 + ca) + sa
    x = x + ga * _A_ref(h, A_k, A_v, A_shift_k, A_ssm_k, A_ssm_D)
    h = _layernorm(x, axis=-1) * (1 + cb) + sb
    x = x + gb * _B_ref(h, B_w1, B_w2, B_w3, B_w4)
    return x
```

```python
import jax
import jax.numpy as jnp
import numpy as np
import jax.experimental.pallas as pl
import jax.experimental.pallas.tpu as pltpu

S, D, F = 2048, 640, 1728
T = 128
NB = S // T
R = 512
NC = S // R
f32, bf16 = jnp.float32, jnp.bfloat16


def _dft_matrices():
    ang = np.pi * np.outer(2 * np.arange(T) + 1, np.arange(T)) / (2 * T)
    fwd = np.concatenate([np.cos(ang), -np.sin(ang)], 0)
    sgn = ((-1.0) ** np.arange(T))[:, None]
    prev = np.concatenate([sgn * np.sin(ang), sgn * np.cos(ang)], 0)
    inv = fwd.T / T
    return fwd.astype(bf16), np.concatenate([prev, fwd], 1).astype(bf16), inv.astype(bf16)


def _unroll(n):
    def run(f):
        for i in range(n):
            f(i)
    return run


def _ln(x):
    m = jnp.mean(x, -1, keepdims=True)
    xc = x - m
    v = jnp.mean(xc * xc, -1, keepdims=True)
    return xc * jax.lax.rsqrt(v + 1e-5)


def _gelu(x):
    u = x * (0.7978845608028654 + (0.7978845608028654 * 0.044715) * (x * x))
    hx = 0.5 * x
    return hx + hx * jnp.tanh(u)


def _dot(a, b):
    return jnp.dot(a, b, preferred_element_type=f32)


def _dot_t(a, b):
    return jax.lax.dot_general(a, b, (((1,), (1,)), ((), ())), preferred_element_type=f32)


def _kernel(sk, sd, c, ff, fk, fi,
            q_h, k_h, v_h, ssm_h, w1_h, w2_h, w3_h, w4_h, wm_h, o_h,
            q, k, v, ssm, w1, w2, w3, w4, wm, o, kp, kv, U, K, x, h, h1, sem):
    pairs = [(ssm_h, ssm), (k_h, k), (v_h, v), (wm_h, wm), (q_h, q),
             (w1_h, w1), (w2_h, w2), (w3_h, w3), (w4_h, w4)]
    cp = [pltpu.make_async_copy(a, b, sem.at[i]) for i, (a, b) in enumerate(pairs)]
    for d in cp:
        d.start()

    cp[0].wait()
    K[0] = _dot_t(ff[...], ssm[:, 0:T])
    for l in range(1, NB):
        K[l] = _dot_t(fk[...], ssm[:, (l - 1) * T:(l + 1) * T])

    cp[1].wait()
    cp[2].wait()
    kp[0:8, :] = jnp.zeros((8, D), f32)

    @_unroll(NB)
    def _(a):
        r = a * T
        kp[pl.ds(r + 8, T), :] = k[pl.ds(r, T), :].astype(f32)

    @_unroll(NB)
    def _(a):
        r = a * T
        acc = kp[pl.ds(r + 8, T), :] * sk[0:1, :].astype(f32)
        for j in range(1, 4):
            acc += kp[pl.ds(r + 8 - j, T), :] * sk[j:j + 1, :].astype(f32)
        p = (acc * v[pl.ds(r, T), :].astype(f32)).astype(bf16)
        kv[pl.ds(r, T), :] = p
        U[a] = _dot(ff[...], p)

    @pl.loop(0, T // 8)
    def _(g):
        r = pl.multiple_of(g * 8, 8)
        for t in range(D // 128):
            ls = slice(t * 128, (t + 1) * 128)
            ur = [U[a, pl.ds(r, 8), ls] for a in range(NB)]
            ui = [U[a, pl.ds(T + r, 8), ls] for a in range(NB)]
            kr = [K[a, pl.ds(r, 8), ls] for a in range(NB)]
            ki = [K[a, pl.ds(T + r, 8), ls] for a in range(NB)]

            def causal(kk, uu, a):
                z = kk[0] * uu[a]
                for l in range(1, a + 1):
                    z = z + kk[l] * uu[a - l]
                return z

            p0 = [causal(kr, ur, a) for a in range(NB)]
            p1 = [causal(ki, ui, a) for a in range(NB)]
            for a in range(NB):
                U[a, pl.ds(r, 8), ls] = p0[a] - p1[a]
            ps = [p0[a] + p1[a] for a in range(NB)]
            us = [ur[a] + ui[a] for a in range(NB)]
            ks = [kr[a] + ki[a] for a in range(NB)]
            for a in range(NB):
                U[a, pl.ds(T + r, 8), ls] = causal(ks, us, a) - ps[a]

    cp[3].wait()
    cf = c[...].astype(f32)
    sc = jnp.broadcast_to(cf * jax.nn.sigmoid(cf), (8, D)).astype(bf16)
    mod = _dot(sc, wm[...])[0:1]
    sa, ca, ga, sb, cb, gb = [mod[:, i * D:(i + 1) * D] for i in range(6)]
    ca1, cb1 = 1 + ca, 1 + cb
    sdf = sd[...].astype(f32)

    cp[4].wait()
    cp[5].wait()
    h1[0:8, :] = jnp.zeros((8, D), f32)
    h1[S + 8:S + 16, :] = jnp.zeros((8, D), f32)

    def stage_a(i):
        r = i * R
        rs = pl.ds(r, R)
        y = jnp.concatenate(
            [_dot(fi[...], U[i * (R // T) + j].astype(bf16)) for j in range(R // T)], 0)
        y = y + kv[rs, :].astype(f32) * sdf
        qq = q[rs, :].astype(f32)
        xx = qq + ga * ((_ln(qq) * ca1 + sa) * y)
        hh = _ln(xx) * cb1 + sb
        x[rs, :] = xx
        h[rs, :] = hh
        h1[pl.ds(r + 8, R), :] = _gelu(_dot(_ln(hh).astype(bf16), w1[...]))

    def stage_b(i):
        r = i * R
        rs = pl.ds(r, R)
        lane = jax.lax.broadcasted_iota(jnp.int32, (R, 128), 1)

        def g(off, t):
            return h1[pl.ds(r + 8 + off, R), t * 128:(t + 1) * 128]

        hs = jnp.concatenate([
            g(-1, 0),
            jnp.where(lane < 32, g(-1, 1), g(1, 1)),
            jnp.where(lane < 64, g(1, 2), g(-2, 2)),
            jnp.where(lane < 96, g(-2, 3), g(2, 3)),
            g(2, 4)], 1).astype(bf16)
        x1 = h[rs, :] + _dot(hs, w2[...])
        m = _gelu(_dot_t(_ln(x1).astype(bf16), w3[...])).astype(bf16)
        o[rs, :] = (x[rs, :] + gb * (x1 + _dot(m, w4[...]))).astype(bf16)
        pltpu.make_async_copy(o.at[rs], o_h.at[rs], sem.at[9]).start()

    stage_a(0)
    stage_a(1)
    for j in (6, 7, 8):
        cp[j].wait()
    for i in range(NC):
        if i + 2 < NC:
            stage_a(i + 2)
        stage_b(i)

    pltpu.make_async_copy(o, o_h, sem.at[9]).wait()


@jax.jit
def pallas_adaLN_cond__ssm_conv_h3__mixer_s_mlp__prompt_kernel(
        A_q, A_k, A_v, A_shift_k, A_ssm_k, A_ssm_D, B_x, B_w1, B_w2, B_w3, B_w4, c, w_mod):
    ff, fk, fi = _dft_matrices()
    vm = pl.BlockSpec(memory_space=pltpu.VMEM)
    hb = pl.BlockSpec(memory_space=pltpu.HBM)
    V = pltpu.VMEM
    out = pl.pallas_call(
        _kernel,
        out_shape=jax.ShapeDtypeStruct((S, D), bf16),
        in_specs=[vm] * 6 + [hb] * 9,
        out_specs=hb,
        scratch_shapes=[
            V((S, D), bf16), V((S, D), bf16), V((S, D), bf16), V((D, S), bf16),
            V((D, D), bf16), V((D, D), bf16), V((F, D), bf16), V((F, D), bf16),
            V((D, 6 * D), bf16), V((S, D), bf16),
            V((S + 8, D), f32), V((S, D), bf16),
            V((NB, 2 * T, D), f32), V((NB, 2 * T, D), f32),
            V((S, D), f32), V((S, D), f32), V((S + 16, D), f32),
            pltpu.SemaphoreType.DMA((10,)),
        ],
        compiler_params=pltpu.CompilerParams(vmem_limit_bytes=110 * 2**20),
    )(A_shift_k.T, A_ssm_D.reshape(1, D), c, ff, fk, fi,
      A_q.reshape(S, D), A_k.reshape(S, D), A_v.reshape(S, D), A_ssm_k,
      B_w1, B_w2, B_w3.T, B_w4, w_mod)
    return out.reshape(1, S, D)
```

```python
import jax
import jax.numpy as jnp
import numpy as np
import jax.experimental.pallas as pl
import jax.experimental.pallas.tpu as pltpu

S, D, F = 2048, 640, 1728
T = 128
NB = S // T
R = 256
UN = 4
NC = S // R
f32, bf16 = jnp.float32, jnp.bfloat16


def _dft_matrices():
    f = np.concatenate([np.arange(0, T, 2), np.arange(1, T, 2)])
    ang = np.pi * np.outer(2 * f + 1, np.arange(T)) / (2 * T)
    fwd = np.concatenate([np.cos(ang), -np.sin(ang)], 0)
    return fwd.astype(bf16), (fwd.T / T).astype(bf16)


def _ln(x):
    m = jnp.mean(x, -1, keepdims=True)
    xc = x - m
    v = jnp.mean(xc * xc, -1, keepdims=True)
    return xc * jax.lax.rsqrt(v + 1e-5)


def _gelu(x):
    u = x * (0.7978845608028654 + (0.7978845608028654 * 0.044715) * (x * x))
    hx = 0.5 * x
    return hx + hx * jnp.tanh(u)


def _dot(a, b):
    return jnp.dot(a, b, preferred_element_type=f32)


def _dot_t(a, b):
    return jax.lax.dot_general(a, b, (((1,), (1,)), ((), ())), preferred_element_type=f32)


def _kernel(sk, sd, c, ff, fi,
            q_h, k_h, v_h, ssm_h, w1_h, w2_h, w3_h, w4_h, wm_h, o_h,
            q, k, v, ssm, w1, w2, w3, w4, wm, o, kv, U, K, x, h, h1, sem, tsem):
    pairs = [(wm_h, wm), (q_h, q), (w1_h, w1), (w2_h, w2), (w3_h, w3), (w4_h, w4)]
    cp = [pltpu.make_async_copy(a, b, sem.at[i]) for i, (a, b) in enumerate(pairs)]
    NT = D // 128
    tc = []
    for t in range(NT):
        ls = pl.ds(t * 128, 128)
        tc.append([
            pltpu.make_async_copy(k_h.at[:, ls], k.at[t, pl.ds(16, S)], tsem.at[3 * t]),
            pltpu.make_async_copy(v_h.at[:, ls], v.at[t], tsem.at[3 * t + 1])] + [
            pltpu.make_async_copy(ssm_h.at[ls, pl.ds(a * T, T)], ssm.at[t, a], tsem.at[3 * t + 2])
            for a in range(NB)])
    for d in tc[0] + tc[1]:
        d.start()
    skf = sk[...].astype(f32)
    sdf = sd[...].astype(f32)
    for t in range(NT):
        k[t, 0:16, :] = jnp.zeros((16, 128), bf16)
        U[t][0] = jnp.zeros((2 * T, 128), f32)

    def gate(t, a):
        r = pl.multiple_of(a * T, T)
        w = skf[:, t * 128:(t + 1) * 128]
        kk = k[t, pl.ds(r, T + 16), :].astype(f32)
        acc = kk[16:] * w[0:1]
        for j in range(1, 4):
            acc += kk[16 - j:16 - j + T] * w[j:j + 1]
        p = (acc * v[t, pl.ds(r, T), :].astype(f32)).astype(bf16)
        kv[t][pl.ds(r, T), :] = p

    def forward(t, a):
        p = kv[t][pl.ds(pl.multiple_of(a * T, T), T), :]
        U[t][a + 1] = _dot(ff[...], p)
        K[t][a] = _dot_t(ff[...], ssm[t, a])

    def causal(kk, uu, a):
        z = kk[0] * uu[a]
        for l in range(1, a + 1):
            z = z + kk[l] * uu[a - l]
        return z

    def mix(t, g):
        re = pl.ds(pl.multiple_of(g * 8, 8), 8)
        im = pl.ds(pl.multiple_of(g * 8 + T, 8), 8)
        n = range(NB)
        ur = [U[t][a + 1, re, :] for a in n]
        kr = [K[t][a, re, :] for a in n]
        p0 = [causal(kr, ur, a) for a in n]
        ui = [U[t][a + 1, im, :] for a in n]
        ki = [K[t][a, im, :] for a in n]
        ps = []
        for a in n:
            p1 = causal(ki, ui, a)
            U[t][a + 1, re, :] = p0[a] - p1
            ps.append(p0[a] + p1)
        us = [ur[a] + ui[a] for a in n]
        ks = [kr[a] + ki[a] for a in n]
        for a in n:
            U[t][a + 1, im, :] = causal(ks, us, a) - ps[a]

    def inverse(t, a):
        H = T // 2
        cur, pre = U[t][a + 1], U[t][a]
        z = jnp.concatenate([
            cur[0:H] - pre[2 * H:3 * H], cur[H:2 * H] + pre[3 * H:],
            cur[2 * H:3 * H] + pre[0:H], cur[3 * H:] - pre[H:2 * H]], 0)
        rs = pl.ds(pl.multiple_of(a * T, T), T)
        ls = slice(t * 128, (t + 1) * 128)
        x[rs, ls] = _dot(fi[...], z.astype(bf16)) + kv[t][rs, :].astype(f32) * sdf[:, ls]

    for p in range(NT + 2):
        if p < NT:
            for d in tc[p]:
                d.wait()
            gate(p, 0)
        if p + 2 < NT:
            for d in tc[p + 2]:
                d.start()
        if p < len(cp):
            cp[p].start()
        if p == NT + 1:
            cp[0].wait()
            cf = c[...].astype(f32)
            sc = jnp.broadcast_to(cf * jax.nn.sigmoid(cf), (8, D)).astype(bf16)
            mod = _dot(sc, wm[...])[0:1]

        @pl.loop(0, NB, unroll=UN)
        def _(a):
            if p < NT:
                forward(p, a)
                gate(p, jnp.minimum(a + 1, NB - 1))
            if 0 <= p - 2:
                inverse(p - 2, a)
            if 0 <= p - 1 < NT:
                mix(p - 1, a)

    sa, ca, ga, sb, cb, gb = [mod[:, i * D:(i + 1) * D] for i in range(6)]
    ca1, cb1 = 1 + ca, 1 + cb

    cp[1].wait()
    cp[2].wait()
    h1[0:8, :] = jnp.zeros((8, D), f32)
    h1[S + 8:S + 16, :] = jnp.zeros((8, D), f32)

    def stage_a(i):
        r = pl.multiple_of(i * R, R)
        rs = pl.ds(r, R)
        y = x[rs, :]
        qq = q[rs, :].astype(f32)
        xx = qq + ga * ((_ln(qq) * ca1 + sa) * y)
        hh = _ln(xx) * cb1 + sb
        x[rs, :] = xx
        h[rs, :] = hh
        h1[pl.ds(r + 8, R), :] = _gelu(_dot(_ln(hh).astype(bf16), w1[...]))

    def stage_b(i):
        r = pl.multiple_of(i * R, R)
        rs = pl.ds(r, R)
        lane = jax.lax.broadcasted_iota(jnp.int32, (R, 128), 1)

        def g(off, t):
            return h1[pl.ds(r, R + 16), t * 128:(t + 1) * 128][8 + off:8 + off + R]

        hs = jnp.concatenate([
            g(-1, 0),
            jnp.where(lane < 32, g(-1, 1), g(1, 1)),
            jnp.where(lane < 64, g(1, 2), g(-2, 2)),
            jnp.where(lane < 96, g(-2, 3), g(2, 3)),
            g(2, 4)], 1).astype(bf16)
        x1 = h[rs, :] + _dot(hs, w2[...])
        m = _gelu(_dot_t(_ln(x1).astype(bf16), w3[...])).astype(bf16)
        o[rs, :] = (x[rs, :] + gb * (x1 + _dot(m, w4[...]))).astype(bf16)
        pltpu.make_async_copy(o.at[rs], o_h.at[rs], sem.at[6]).start()

    pl.loop(0, 2)(stage_a)
    for j in (3, 4, 5):
        cp[j].wait()

    @pl.loop(0, NC - 2)
    def _(i):
        stage_b(i)
        stage_a(i + 2)

    pl.loop(NC - 2, NC)(stage_b)

    pltpu.make_async_copy(o, o_h, sem.at[6]).wait()


@jax.jit
def pallas_adaLN_cond__ssm_conv_h3__mixer_s_mlp__prompt_kernel(
        A_q, A_k, A_v, A_shift_k, A_ssm_k, A_ssm_D, B_x, B_w1, B_w2, B_w3, B_w4, c, w_mod):
    ff, fi = _dft_matrices()
    vm = pl.BlockSpec(memory_space=pltpu.VMEM)
    hb = pl.BlockSpec(memory_space=pltpu.HBM)
    V = pltpu.VMEM
    out = pl.pallas_call(
        _kernel,
        out_shape=jax.ShapeDtypeStruct((S, D), bf16),
        in_specs=[vm] * 5 + [hb] * 9,
        out_specs=hb,
        scratch_shapes=[
            V((S, D), bf16), V((5, S + 16, 128), bf16), V((5, S, 128), bf16),
            V((5, NB, 128, T), bf16),
            V((D, D), bf16), V((D, D), bf16), V((F, D), bf16), V((F, D), bf16),
            V((D, 6 * D), bf16), V((S, D), bf16),
            [V((S, 128), bf16)] * 5,
            [V((NB + 1, 2 * T, 128), f32)] * 5, [V((NB, 2 * T, 128), f32)] * 5,
            V((S, D), f32), V((S, D), f32), V((S + 16, D), f32),
            pltpu.SemaphoreType.DMA((7,)), pltpu.SemaphoreType.DMA((15,)),
        ],
        compiler_params=pltpu.CompilerParams(vmem_limit_bytes=110 * 2**20),
    )(A_shift_k.T, A_ssm_D.reshape(1, D), c, ff, fi,
      A_q.reshape(S, D), A_k.reshape(S, D), A_v.reshape(S, D), A_ssm_k,
      B_w1, B_w2, B_w3.T, B_w4, w_mod)
    return out.reshape(1, S, D)
```
